```python
import os as _os
_os.environ.setdefault('JAX_PLATFORMS', 'cpu')
import jax
import jax.numpy as jnp

def _softmax(x, axis=-1):
    return jax.nn.softmax(x, axis=axis)

def _gelu(x):
    return jax.nn.gelu(x, approximate=True)

def _silu(x):
    return jax.nn.silu(x)

def _sigmoid(x):
    return jax.nn.sigmoid(x)

def _layernorm(x, axis=-1, eps=1e-05):
    m = jnp.mean(x, axis=axis, keepdims=True)
    v = jnp.var(x, axis=axis, keepdims=True)
    return (x - m) / jnp.sqrt(v + eps)

def _scatter_add(tgt, idx, src, axis=0):
    return tgt.at[idx].add(src)

def _segment_sum(src, seg, n):
    return jax.ops.segment_sum(src, seg, n)

class _Rng:

    def __init__(self, key):
        self._k = key

    def _next(self):
        self._k, sub = jax.random.split(self._k)
        return sub

    def normal(self, shape):
        return jax.random.normal(self._next(), shape, dtype=jnp.bfloat16)

    def randint(self, lo, hi, shape):
        return jax.random.randint(self._next(), shape, lo, hi, dtype=jnp.int32)

    def uniform(self, shape, lo=0.0, hi=1.0):
        return jax.random.uniform(self._next(), shape, jnp.bfloat16, lo, hi)

    def permutation(self, n):
        return jax.random.permutation(self._next(), n)
kernel_name = 'recurrent_scan__memory_aug_recurrent_mem_tr__mixer_gmlp__prompt'

def setup_inputs():
    _rng = _Rng(jax.random.key(int.from_bytes(__import__("os").urandom(4), "little")))
    _w = lambda a: (lambda t: t.astype(jnp.bfloat16) if jnp.issubdtype(t.dtype, jnp.floating) else t)(jnp.asarray(a))

    def _A_setup():
        B, S, Dm = (1, 2048, 640)
        H, Dh = (32, 128)
        M, seg = (8, 32)
        seg = min(seg, S)
        S = S // seg * seg
        return {'x': _w((lambda *s: _rng.normal(s) * 0.05)(B, S, Dm)), 'mem0': _w((lambda *s: _rng.normal(s) * 0.1)(B, M, Dm)), 'Wq': _w((lambda *s: _rng.normal(s) * 1.6)(Dm, H, Dh) * Dm ** (-0.5)), 'Wk': _w((lambda *s: _rng.normal(s) * 1.6)(Dm, H, Dh) * Dm ** (-0.5)), 'Wv': _w((lambda *s: _rng.normal(s) * 0.1)(Dm, H, Dh) * Dm ** (-0.5)), 'Wo': _w((lambda *s: _rng.normal(s) * 0.1)(H, Dh, Dm) * (H * Dh) ** (-0.5)), 'seg_len': seg}
    _A_in = _A_setup()

    def _B_setup():
        B, S, D, F = (1, 2048, 640, 1728)
        Fh = F // 2
        return {'x': _w((lambda *s: _rng.normal(s) * 0.05)(B, S, D)), 'w_in': _w((lambda *s: _rng.normal(s) * 0.8)(D, 2 * Fh)), 'w_sp': _w(0.01 * (lambda *s: _rng.normal(s) * 0.8)(S, S)), 'b_sp': _w(1.0 + 0.01 * (lambda *s: _rng.normal(s) * 0.05)(S)), 'w_out': _w((lambda *s: _rng.normal(s) * 0.05)(Fh, D))}
    _B_in = _B_setup()
    return {'A_x': _A_in['x'], 'A_mem0': _A_in['mem0'], 'A_Wq': _A_in['Wq'], 'A_Wk': _A_in['Wk'], 'A_Wv': _A_in['Wv'], 'A_Wo': _A_in['Wo'], 'A_seg_len': _A_in['seg_len'], 'B_x': _B_in['x'], 'B_w_in': _B_in['w_in'], 'B_w_sp': _B_in['w_sp'], 'B_b_sp': _B_in['b_sp'], 'B_w_out': _B_in['w_out']}

def reference(A_x, A_mem0, A_Wq, A_Wk, A_Wv, A_Wo, A_seg_len, B_x, B_w_in, B_w_sp, B_b_sp, B_w_out):

    def _A_ref(x, mem0, Wq, Wk, Wv, Wo, seg_len):
        B, S, Dm = x.shape
        H, Dh = (Wq.shape[1], Wq.shape[2])
        M = mem0.shape[1]
        scale = Dh ** (-0.5)
        n_seg = S // seg_len
        L = M + seg_len
        idx = jnp.arange(L)
        mask = (idx[:, None] < M) | (idx[:, None] >= idx[None, :])
        mem = mem0
        outs = []
        for s in range(n_seg):
            xs = x[:, s * seg_len:(s + 1) * seg_len, :].copy()
            h = jnp.concatenate([mem, xs], axis=1)
            q = jnp.einsum('btd,dhe->bhte', h, Wq)
            k = jnp.einsum('btd,dhe->bhte', h, Wk)
            v = jnp.einsum('btd,dhe->bhte', h, Wv)
            scores = jnp.einsum('bhqe,bhke->bhqk', q, k) * scale
            scores = jnp.where(mask[None, None], scores, -1000000000.0)
            p = _softmax(scores, axis=-1)
            o = jnp.einsum('bhqk,bhke->bhqe', p, v)
            o = jnp.einsum('bhte,hed->btd', o, Wo)
            mem = o[:, :M, :].copy()
            outs.append(o[:, M:, :])
        return jnp.concatenate(outs, axis=1)

    def _B_ref(x, w_in, w_sp, b_sp, w_out):
        B, S, D = x.shape
        F = w_in.shape[-1]
        Fh = F // 2
        z = _gelu(jnp.einsum('bsd,df->bsf', x, w_in))
        z1 = z[..., :Fh].copy()
        z2 = _layernorm(z[..., Fh:], axis=-1)
        g = jnp.einsum('ts,bsf->btf', w_sp, z2) + b_sp[None, :, None]
        return jnp.einsum('bsf,fd->bsd', z1 * g, w_out)
    x = A_x
    xn = _layernorm(x, axis=-1)
    s = _A_ref(xn, A_mem0, A_Wq, A_Wk, A_Wv, A_Wo, A_seg_len)
    g = _silu(_B_ref(xn, B_w_in, B_w_sp, B_b_sp, B_w_out))
    return x + s * g
```

```python
import jax
import jax.numpy as jnp
from jax import lax
import jax.experimental.pallas as pl
import jax.experimental.pallas.tpu as pltpu

F32 = jnp.float32
BF16 = jnp.bfloat16
U32 = jnp.uint32

S, D, H, E, M, SEG = 2048, 640, 32, 128, 8, 32
L = M + SEG
NSEG = S // SEG
FH = 864
EPS = 1e-5
SK1 = 1
SK2 = 3
UN = 4
NB = 8
RB = S // NB
DB = D // NB
OB = H * E // NB

SEM_X = 0
SEM_WIN = SEM_X + NB
SEM_GRP = SEM_WIN + 1
SEM_WOUT = SEM_GRP + 5 * NB
SEM_MEM = SEM_WOUT + 1
SEM_B = SEM_MEM + 1
SEM_OUT = SEM_B + 1
NSEM = SEM_OUT + NSEG // UN


def _dot(a, b):
    return lax.dot_general(a, b, (((1,), (0,)), ((), ())), preferred_element_type=F32)


def _dot_nt(a, b):
    return lax.dot_general(a, b, (((1,), (1,)), ((), ())), preferred_element_type=F32)


def _ln(x):
    m = jnp.mean(x, axis=-1, keepdims=True)
    c = x - m
    v = jnp.mean(c * c, axis=-1, keepdims=True)
    return c * lax.rsqrt(v + EPS)


def _gelu(x):
    return 0.5 * x * (1.0 + jnp.tanh(0.7978845608028654 * (x + 0.044715 * (x * x * x))))


def _recip(l):
    r = pl.reciprocal(l, approx=True)
    return r * (2.0 - l * r)


def _kernel(x_hbm, mem0_hbm, wq_hbm, wk_hbm, wv_hbm, wo_hbm, win_hbm, wsp_hbm, bsp_hbm, wout_hbm,
            out_hbm,
            x_s, xn_s, raw_s, wqkv_s, wo_s, win_s, wsp_s, wout_s,
            z1_s, z2_u, mem0_s, bsp_s, bcol_s, out_s, sems):
    z2_s = z2_u.bitcast(BF16)
    wqkv_u = wqkv_s.bitcast(U32)
    wo_u = wo_s.bitcast(U32)
    wsp_u = wsp_s.bitcast(U32)
    wout_u = wout_s.bitcast(U32)

    def cat_tiles(ref_u, n, rows):
        return jnp.concatenate([pltpu.bitcast(ref_u[j, rows, :], BF16) for j in range(n)], axis=1)

    def x_copy(c):
        return pltpu.make_async_copy(x_hbm.at[pl.ds(c * RB, RB), :], x_s.at[pl.ds(c * RB, RB), :], sems.at[SEM_X + c])

    def grp_copies(i):
        cs = []
        for wi, w_hbm in enumerate((wq_hbm, wk_hbm, wv_hbm)):
            cs.append(pltpu.make_async_copy(w_hbm.at[pl.ds(i * DB * H, DB * H), :],
                                            raw_s.at[wi, pl.ds(i * DB * H, DB * H), :],
                                            sems.at[SEM_GRP + 5 * i + 1 + wi]))
        return cs

    wsp_copies = [pltpu.make_async_copy(wsp_hbm.at[:, pl.ds(j * 128, 128)], wsp_s.at[j], sems.at[SEM_GRP])
                  for j in range(S // 128)]
    late_copies = [pltpu.make_async_copy(wout_hbm.at[:, pl.ds(j * 128, 128)], wout_s.at[j], sems.at[SEM_WOUT])
                   for j in range(D // 128)]
    late_copies += [pltpu.make_async_copy(wo_hbm.at[:, pl.ds(j * 128, 128)], wo_s.at[j], sems.at[SEM_WOUT])
                    for j in range(D // 128)]

    def out_copy(i):
        n = UN * SEG
        return pltpu.make_async_copy(out_s.at[pl.ds(i * n, n), :], out_hbm.at[pl.ds(i * n, n), :],
                                     sems.at[SEM_OUT + i])

    b_copy = pltpu.make_async_copy(bsp_hbm, bsp_s, sems.at[SEM_B])
    mem_copy = pltpu.make_async_copy(mem0_hbm, mem0_s, sems.at[SEM_MEM])
    win_copy = pltpu.make_async_copy(win_hbm, win_s, sems.at[SEM_WIN])

    b_copy.start()
    x_copy(0).start()
    win_copy.start()
    for c in range(1, NB):
        x_copy(c).start()
    mem_copy.start()
    for cp in wsp_copies:
        cp.start()

    b_copy.wait()
    eye = lax.broadcasted_iota(jnp.int32, (128, 128), 0) == lax.broadcasted_iota(jnp.int32, (128, 128), 1)
    b2 = bsp_s[...].astype(F32)
    for c in range(S // 128):
        row = jnp.broadcast_to(b2[c:c + 1, :], (128, 128))
        col = jnp.sum(jnp.where(eye, row, 0.0), axis=1, keepdims=True)
        bcol_s[c * 128:(c + 1) * 128, :] = jnp.broadcast_to(col, (128, 128))

    x_copy(0).wait()
    xn_s[0:RB, :] = _ln(x_s[0:RB, :].astype(F32))
    win_copy.wait()

    def phase1(c, carry):
        @pl.when(c < NB - 1)
        def _():
            x_copy(c + 1).wait()
        for cp in grp_copies(c):
            cp.start()
        r = pl.multiple_of(c * RB, RB)
        xb = xn_s[pl.ds(r, RB), :].astype(BF16)
        z2 = _ln(_gelu(_dot_nt(xb, win_s[FH:, :])))
        z2_s[pl.ds(r, RB), :] = z2.astype(BF16)
        z1_s[pl.ds(r, RB), :] = _gelu(_dot_nt(xb, win_s[:FH, :]))
        rn = pl.multiple_of(jnp.minimum(c + 1, NB - 1) * RB, RB)
        xn_s[pl.ds(rn, RB), :] = _ln(x_s[pl.ds(rn, RB), :].astype(F32))
        return carry
    lax.fori_loop(0, NB, phase1, 0)
    for cp in late_copies:
        cp.start()
    for cp in wsp_copies:
        cp.wait()

    raw32 = raw_s.bitcast(U32)

    def phase2(i, carry):
        for cp in grp_copies(i):
            cp.wait()
        r = pl.multiple_of(i * RB, RB)
        rh = pl.multiple_of(i * (RB // 2), RB // 2)
        g = _dot(cat_tiles(wsp_u, S // 128, pl.ds(rh, RB // 2)), z2_s[...]) + bcol_s[pl.ds(r, RB), 0:1]
        z1_s[pl.ds(r, RB), :] = z1_s[pl.ds(r, RB), :] * g
        base = pl.multiple_of(i * (DB * H // 2), DB * H // 2)
        dbase = pl.multiple_of(i * DB, DB)
        for wi in range(3):
            blk = raw32.at[wi, pl.ds(base, DB * H // 2), :]
            for j in range(H // 2):
                xw = blk[pl.ds(j, DB, stride=H // 2), :]
                lo = pltpu.bitcast(xw << 16, F32).astype(BF16)
                hi = pltpu.bitcast(xw & jnp.uint32(0xFFFF0000), F32).astype(BF16)
                wqkv_s[6 * j + wi, pl.ds(dbase, DB), :] = lo
                wqkv_s[6 * j + 3 + wi, pl.ds(dbase, DB), :] = hi
        return carry
    lax.fori_loop(0, NB, phase2, 0)

    for cp in late_copies:
        cp.wait()
    mem_copy.wait()

    scale = E ** -0.5
    qi = lax.broadcasted_iota(jnp.int32, (L, L), 0)
    ki = lax.broadcasted_iota(jnp.int32, (L, L), 1)
    mask = (qi < M) | (qi >= ki)

    def step(s, mem):
        r0 = pl.multiple_of(s * SEG, SEG)
        qkv = [None] * H
        ps = [None] * H
        outs = [None] * H

        def proj(hd):
            qkv[hd] = _dot(h, jnp.concatenate([pltpu.bitcast(wqkv_u[3 * hd + wi], BF16) for wi in range(3)], axis=1))

        def scores(hd):
            q = qkv[hd][:, :E]
            k = qkv[hd][:, E:2 * E]
            sc = _dot_nt(q, k) * scale
            sc = jnp.where(mask, sc, -1e9)
            mx = jnp.max(sc, axis=-1, keepdims=True)
            p = jnp.exp(sc - mx)
            l = jnp.sum(p, axis=-1, keepdims=True)
            ps[hd] = (p, l)

        def pv(hd):
            p, l = ps[hd]
            v = qkv[hd][:, 2 * E:]
            outs[hd] = _dot(p, v) * _recip(l)

        def wo(a, b):
            return _dot(jnp.concatenate(outs[a:b], axis=1), cat_tiles(wo_u, D // 128, pl.ds(a * E // 2, (b - a) * E // 2)))

        bo = _dot(z1_s[pl.ds(r0, SEG), :], cat_tiles(wout_u, D // 128, pl.ds(0, FH // 2)))
        gate = bo * jax.nn.sigmoid(bo)
        h = jnp.concatenate([mem, xn_s[pl.ds(r0, SEG), :]], axis=0)
        for hd in range(H):
            proj(hd)
            if hd >= SK1:
                scores(hd - SK1)
            if hd >= SK2:
                pv(hd - SK2)
        y = None
        a = 0
        for t in range(H, H + SK2):
            part = wo(a, a + 4)
            a += 4
            y = part if y is None else y + part
            if t - SK1 < H:
                scores(t - SK1)
            pv(t - SK2)
        y = y + wo(a, H - 4)
        y = y + wo(H - 4, H)
        out_s[pl.ds(r0, SEG), :] = (x_s[pl.ds(r0, SEG), :].astype(F32) + y[M:] * gate).astype(BF16)
        return y[:M]

    def stepu(i, mem):
        for j in range(UN):
            mem = step(i * UN + j, mem)
        out_copy(i).start()
        return mem
    lax.fori_loop(0, NSEG // UN, stepu, mem0_s[...].astype(F32))
    for i in range(NSEG // UN):
        out_copy(i).wait()


def pallas_recurrent_scan__memory_aug_recurrent_mem_tr__mixer_gmlp__prompt_kernel(
    A_x, A_mem0, A_Wq, A_Wk, A_Wv, A_Wo, A_seg_len, B_x, B_w_in, B_w_sp, B_b_sp, B_w_out):
    hbm = pl.BlockSpec(memory_space=pltpu.HBM)
    out = pl.pallas_call(
        _kernel,
        out_shape=jax.ShapeDtypeStruct((S, D), BF16),
        in_specs=[hbm] * 10,
        out_specs=hbm,
        scratch_shapes=[
            pltpu.VMEM((S, D), BF16),
            pltpu.VMEM((S, D), F32),
            pltpu.VMEM((3, D * H, E), BF16),
            pltpu.VMEM((3 * H, D, E), BF16),
            pltpu.VMEM((D // 128, H * E, 128), BF16),
            pltpu.VMEM((2 * FH, D), BF16),
            pltpu.VMEM((S // 128, S, 128), BF16),
            pltpu.VMEM((D // 128, FH, 128), BF16),
            pltpu.VMEM((S, FH), F32),
            pltpu.VMEM((S // 2, FH), U32),
            pltpu.VMEM((M, D), BF16),
            pltpu.VMEM((S // 128, 128), BF16),
            pltpu.VMEM((S, 128), F32),
            pltpu.VMEM((S, D), BF16),
            pltpu.SemaphoreType.DMA((NSEM,)),
        ],
        compiler_params=pltpu.CompilerParams(vmem_limit_bytes=120 * 1024 * 1024),
    )(A_x.reshape(S, D), A_mem0.reshape(M, D), A_Wq.reshape(D * H, E), A_Wk.reshape(D * H, E),
      A_Wv.reshape(D * H, E), A_Wo.reshape(H * E, D), B_w_in.T, B_w_sp, B_b_sp.reshape(S // 128, 128), B_w_out)
    return out.reshape(1, S, D)
```

```python
import jax
import jax.numpy as jnp
from jax import lax
import jax.experimental.pallas as pl
import jax.experimental.pallas.tpu as pltpu

F32 = jnp.float32
BF16 = jnp.bfloat16
U32 = jnp.uint32

S, D, H, E, M, SEG = 2048, 640, 32, 128, 8, 32
L = M + SEG
NSEG = S // SEG
FH = 864
EPS = 1e-5

SK1 = 2
SK2 = 6
UN = 128 // SEG
NB = 4
RB = S // NB
TPB = RB // 128
NXC = 8
XC = S // NXC
XPB = RB // XC
NB2 = 4
TPB2 = S // NB2 // 128
DB = D // NB2
PB = DB // 2
PITCH = D // 2 + 4
NT = S // 128
KD = D // 128
MCH = [(0, 256), (256, 256), (512, 256), (768, 96)]
MCH0 = [(0, 224), (224, 208), (432, 208), (640, 224)]
WPIECES = [(FH, 224), (FH + 224, 416), (FH + 640, 224), (0, FH)]
WGROUP = [0, 1, 2, 2]
NWP = 3

SEM_X = 0
SEM_WIN = SEM_X + NXC
SEM_GRP = SEM_WIN + NWP
SEM_WSP = SEM_GRP + NB2
SEM_LATE = SEM_WSP + 1
SEM_OUT = SEM_LATE + 1
NSEM = SEM_OUT + 1


def _slab(hd):
    return ((hd % 2) * 2 + hd // 16) * 8 + (hd % 16) // 2


def _dot(a, b):
    return lax.dot_general(a, b, (((1,), (0,)), ((), ())), preferred_element_type=F32)


def _dot_nt(a, b):
    return lax.dot_general(a, b, (((1,), (1,)), ((), ())), preferred_element_type=F32)


def _ln(x):
    m = jnp.mean(x, axis=-1, keepdims=True)
    c = x - m
    v = jnp.mean(c * c, axis=-1, keepdims=True)
    return c * lax.rsqrt(v + EPS)


def _gelu(x):
    t = jnp.tanh(x * (0.7978845608028654 + (0.7978845608028654 * 0.044715) * (x * x)))
    hx = 0.5 * x
    return hx + hx * t


def _recip(l):
    r = pl.reciprocal(l, approx=True)
    return r * (2.0 - l * r)


def _kernel(x_hbm, mem0_hbm, wq_hbm, wk_hbm, wv_hbm, wo_hbm, win_hbm, wsp_hbm, bsp_hbm, wout_hbm,
            out_hbm,
            x_s, xn_s, raw_s, wqkv_s, wo_s, win_s, wsp_s, wout_s,
            z1_s, y_s, z2_s, u_s, mem0_s, bsp_s, b32_s, out_s, st_s, sems):
    wqkv_u = wqkv_s.bitcast(U32)
    wo_u = wo_s.bitcast(U32)
    win_u = win_s.bitcast(U32)
    wout_u = wout_s.bitcast(U32)
    z2_u = z2_s.bitcast(U32)
    raw_u = raw_s.bitcast(U32)

    def cat_tiles(ref_u, n, lo, rows):
        return jnp.concatenate(
            [pltpu.bitcast(ref_u[j, pl.ds(lo // 2, rows // 2), :], BF16) for j in range(n)], axis=1)

    def x_copy(c):
        return pltpu.make_async_copy(x_hbm.at[pl.ds(c * XC, XC), :], x_s.at[pl.ds(c * XC, XC), :],
                                     sems.at[SEM_X + c])

    def win_copies(grp):
        return [pltpu.make_async_copy(win_hbm.at[pl.ds(lo, n), pl.ds(j * 128, 128)],
                                      win_s.at[j, pl.ds(lo, n), :], sems.at[SEM_WIN + grp])
                for (lo, n), g in zip(WPIECES, WGROUP) if g == grp for j in range(KD)]

    def grp_copies(i):
        return [pltpu.make_async_copy(w_hbm.at[pl.ds(i * DB * H, DB * H), :],
                                      raw_s.at[wi, pl.ds(i * DB * H, DB * H), :], sems.at[SEM_GRP + i])
                for wi, w_hbm in enumerate((wq_hbm, wk_hbm, wv_hbm))]

    wsp_copies = [pltpu.make_async_copy(wsp_hbm, wsp_s, sems.at[SEM_WSP]),
                  pltpu.make_async_copy(bsp_hbm, bsp_s, sems.at[SEM_WSP])]
    late_copies = [pltpu.make_async_copy(wout_hbm.at[:, pl.ds(j * 128, 128)], wout_s.at[j], sems.at[SEM_LATE])
                   for j in range(KD)]
    late_copies += [pltpu.make_async_copy(wo_hbm.at[:, pl.ds(j * 128, 128)], wo_s.at[j], sems.at[SEM_LATE])
                    for j in range(KD)]
    late_copies += [pltpu.make_async_copy(mem0_hbm, mem0_s, sems.at[SEM_LATE])]

    def out_copy(i):
        return pltpu.make_async_copy(out_s.at[pl.ds(i * 128, 128), :], out_hbm.at[pl.ds(i * 128, 128), :],
                                     sems.at[SEM_OUT])

    for c in range(XPB):
        x_copy(c).start()
    for grp in range(NWP):
        for cp in win_copies(grp):
            cp.start()
    for c in range(XPB, NXC):
        x_copy(c).start()
    for cp in wsp_copies:
        cp.start()

    def ln_rows(lo, n):
        xn = _ln(x_s[pl.ds(lo, n), :].astype(F32))
        xn_s[pl.ds(lo, n), :] = xn
        return xn.astype(BF16)

    def z2_chunk(xb, t0, nt, k, lo, n):
        z = _gelu(_dot_nt(cat_tiles(win_u, KD, FH + lo, n), xb))
        for t in range(nt):
            y_s[t0 + t, lo:lo + n, :] = z[:, t * 128:(t + 1) * 128]
        z3 = z.reshape(n // 8, 8, nt * 128)
        st_s[0, k, :, t0 * 128:(t0 + nt) * 128] = jnp.sum(z3, axis=0)
        st_s[1, k, :, t0 * 128:(t0 + nt) * 128] = jnp.sum(z3 * z3, axis=0)

    def z1_half(c):
        xb = xn_s[pl.ds(pl.multiple_of(c * RB, RB), RB), :].astype(BF16)
        m = jnp.sum(jnp.sum(st_s[0], axis=0), axis=0, keepdims=True) * (1.0 / FH)
        s2 = jnp.sum(jnp.sum(st_s[1], axis=0), axis=0, keepdims=True) * (1.0 / FH)
        r = lax.rsqrt(jnp.maximum(s2 - m * m, 0.0) + EPS)
        mr = m * r
        pieces = [(t, hf) for t in range(TPB) for hf in range(2)]
        hf_rows = FH // 2
        for lo, n in MCH:
            z = _gelu(_dot_nt(cat_tiles(win_u, KD, lo, n), xb))
            for t in range(TPB):
                z1_s[c * TPB + t, lo:lo + n, :] = z[:, t * 128:(t + 1) * 128]
                if pieces:
                    z2_s[0, FH:FH + 16, :] = z[0:16, t * 128:(t + 1) * 128].astype(BF16)
                    tp, hf = pieces.pop(0)
                    sl = slice(tp * 128, (tp + 1) * 128)
                    rows = slice(hf * hf_rows, (hf + 1) * hf_rows)
                    z2_s[c * TPB + tp, rows, :] = (y_s[tp, rows, :] * r[:, sl] - mr[:, sl]).astype(BF16)

    xbs = []
    for c in range(XPB):
        x_copy(c).wait()
        xbs.append(ln_rows(c * XC, XC))
    xb0 = jnp.concatenate(xbs, axis=0)
    for k, (lo, n) in enumerate(MCH0):
        grp = {0: 0, 1: 1, 3: 2}.get(k)
        if grp is not None:
            for cp in win_copies(grp):
                cp.wait()
        z2_chunk(xb0, 0, TPB, k, lo, n)

    def phase1_body(c, carry):
        for cc in range(XPB):
            x_copy((c + 1) * XPB + cc).wait()
        for cp in grp_copies(c):
            cp.start()
        z1_half(c)
        for t in range(TPB):
            xb = ln_rows(pl.multiple_of((c + 1) * RB + t * 128, 128), 128)
            for k, (lo, n) in enumerate(MCH):
                z2_chunk(xb, t, 1, k, lo, n)
        return c + 1

    z1_half(lax.fori_loop(0, NB - 1, phase1_body, 0))
    for i in range(NB - 1, NB2):
        for cp in grp_copies(i):
            cp.start()
    for cp in late_copies:
        cp.start()
    for cp in wsp_copies:
        cp.wait()
    b32_s[...] = bsp_s[...].astype(F32)

    def phase2_body(i, carry):
        for cp in grp_copies(i):
            cp.wait()
        dst = wqkv_u.at[pl.ds(pl.multiple_of(i * PB, PB), (3 * H - 1) * PITCH + PB), :]

        def relayout(units):
            for wi, p in units:
                src = raw_u.at[wi, pl.ds(pl.multiple_of(i * PB * H, PB * H), PB * H), :]
                for hi in range(2):
                    wa = src[pl.ds(p * H + hi * 8, 8), :]
                    wb = src[pl.ds(p * H + 16 + hi * 8, 8), :]
                    dst[pl.ds((wi * H + hi * 8) * PITCH + p, 8, stride=PITCH), :] = (
                        (wa & jnp.uint32(0xFFFF)) | (wb << 16))
                    dst[pl.ds((wi * H + 16 + hi * 8) * PITCH + p, 8, stride=PITCH), :] = (
                        (wa >> 16) | (wb & jnp.uint32(0xFFFF0000)))

        units = [(wi, p) for wi in range(3) for p in range(PB)]
        nslot = TPB2 * len(MCH) - 2
        per = -(-len(units) // nslot)
        slot = 0
        for t in range(TPB2):
            tt = i * TPB2 + t
            brow = b32_s[pl.ds(tt, 1), :]
            for lo, n in MCH:
                g = _dot_nt(cat_tiles(z2_u, NT, lo, n), wsp_s[pl.ds(pl.multiple_of(tt * 128, 128), 128), :]) + brow
                z1_s[tt, lo:lo + n, :] = z1_s[tt, lo:lo + n, :] * g
                if slot < nslot:
                    wqkv_u[D // 2:D // 2 + 4, :] = pltpu.bitcast(g[n - 8:n - 4, :], U32)
                    relayout(units[slot * per:(slot + 1) * per])
                slot += 1
        return carry

    lax.fori_loop(0, NB2, phase2_body, 0)
    for cp in late_copies:
        cp.wait()

    scale = E ** -0.5
    qi = lax.broadcasted_iota(jnp.int32, (L, L), 0)
    ki = lax.broadcasted_iota(jnp.int32, (L, L), 1)
    mask = (qi < M) | (qi >= ki)

    def segment(s, j, mem):
        r0 = pl.multiple_of(s * SEG, SEG)
        qkv = [None] * H
        ps = [None] * H
        outs = [None] * H

        def proj(hd):
            w = jnp.concatenate(
                [pltpu.bitcast(wqkv_u[pl.ds((wi * H + _slab(hd)) * PITCH, D // 2), :], BF16) for wi in range(3)],
                axis=1)
            qkv[hd] = _dot(h, w)

        def scores(hd):
            sc = _dot_nt(qkv[hd][:, :E], qkv[hd][:, E:2 * E]) * scale
            sc = jnp.where(mask, sc, -1e9)
            p = jnp.exp(sc - jnp.max(sc, axis=-1, keepdims=True))
            ps[hd] = p * _recip(jnp.sum(p, axis=-1, keepdims=True))

        def pv(hd):
            outs[hd] = _dot(ps[hd], qkv[hd][:, 2 * E:])

        def wo(a, b):
            return _dot(jnp.concatenate(outs[a:b], axis=1), cat_tiles(wo_u, KD, a * E, (b - a) * E))

        def silu_gate():
            bo = _dot(u_s[j * SEG:(j + 1) * SEG, :], cat_tiles(wout_u, KD, 0, FH))
            return bo * jax.nn.sigmoid(bo)

        if j > 0:
            gate = silu_gate()
        h = jnp.concatenate([mem, xn_s[pl.ds(r0, SEG), :]], axis=0)
        for hd in range(H):
            proj(hd)
            if hd >= SK1:
                scores(hd - SK1)
            if hd >= SK2:
                pv(hd - SK2)
        y = None
        a = 0
        for t in range(H, H + SK2):
            part = wo(a, a + 4)
            a += 4
            y = part if y is None else y + part
            if t - SK1 < H:
                scores(t - SK1)
            pv(t - SK2)
        y = y + wo(a, H - 4)
        if j == 0:
            gate = silu_gate()
        y = y + wo(H - 4, H)
        out_s[pl.ds(r0, SEG), :] = (x_s[pl.ds(r0, SEG), :].astype(F32) + y[M:] * gate).astype(BF16)
        return y[:M]

    def phase3_body(i, mem):
        for q in range(0, FH, 128):
            w = min(128, FH - q)
            u_s[:, q:q + w] = z1_s[i, q:q + w, :].T
        for j in range(UN):
            mem = segment(i * UN + j, j, mem)
        out_copy(i).start()
        return mem

    lax.fori_loop(0, NT, phase3_body, mem0_s[...].astype(F32))
    for i in range(NT):
        out_copy(i).wait()


def pallas_recurrent_scan__memory_aug_recurrent_mem_tr__mixer_gmlp__prompt_kernel(
    A_x, A_mem0, A_Wq, A_Wk, A_Wv, A_Wo, A_seg_len, B_x, B_w_in, B_w_sp, B_b_sp, B_w_out,
):
    assert A_x.shape == (1, S, D) and A_Wq.shape == (D, H, E) and B_w_in.shape == (D, 2 * FH)
    if isinstance(A_seg_len, int):
        assert A_seg_len == SEG
    hbm = pl.BlockSpec(memory_space=pl.ANY)
    out = pl.pallas_call(
        _kernel,
        out_shape=jax.ShapeDtypeStruct((S, D), BF16),
        in_specs=[hbm] * 10,
        out_specs=hbm,
        scratch_shapes=[
            pltpu.VMEM((S, D), BF16),
            pltpu.VMEM((S, D), F32),
            pltpu.VMEM((3, D * H, E), BF16),
            pltpu.VMEM((3 * H * PITCH * 2, E), BF16),
            pltpu.VMEM((KD, H * E, 128), BF16),
            pltpu.VMEM((KD, 2 * FH, 128), BF16),
            pltpu.VMEM((S, S), BF16),
            pltpu.VMEM((KD, FH, 128), BF16),
            pltpu.VMEM((NT, FH, 128), F32),
            pltpu.VMEM((TPB, FH, 128), F32),
            pltpu.VMEM((NT, FH + 16, 128), BF16),
            pltpu.VMEM((128, FH), F32),
            pltpu.VMEM((M, D), BF16),
            pltpu.VMEM((NT, 128), BF16),
            pltpu.VMEM((NT, 128), F32),
            pltpu.VMEM((S, D), BF16),
            pltpu.VMEM((2, len(MCH), 8, RB), F32),
            pltpu.SemaphoreType.DMA((NSEM,)),
        ],
        compiler_params=pltpu.CompilerParams(vmem_limit_bytes=120 * 1024 * 1024, disable_bounds_checks=True),
    )(A_x.reshape(S, D), A_mem0.reshape(M, D), A_Wq.reshape(D * H, E), A_Wk.reshape(D * H, E),
      A_Wv.reshape(D * H, E), A_Wo.reshape(H * E, D), B_w_in.T, B_w_sp, B_b_sp.reshape(NT, 128), B_w_out)
    return out.reshape(1, S, D)
```

```python
import jax
import jax.numpy as jnp
from jax import lax
import jax.experimental.pallas as pl
import jax.experimental.pallas.tpu as pltpu

F32 = jnp.float32
BF16 = jnp.bfloat16
U32 = jnp.uint32

S, D, H, E, M, SEG = 2048, 640, 32, 128, 8, 32
L = M + SEG
FH = 864
EPS = 1e-5
LOG2E = 1.4426950408889634

SK1 = 2
SK2 = 6
SKV = 5
KVN = 16
UN = 128 // SEG
NT = S // 128
KD = D // 128

NB = 4
RB = S // NB
TPB = RB // 128
MCH = [(0, 256), (256, 256), (512, 256), (768, 96)]
MCH0 = [(0, 288), (288, 192), (480, 192), (672, 192)]
WPIECES = [(FH, 288), (FH + 288, FH - 288), (0, FH)]

NB2 = 4
TPB2 = NT // NB2
DB = D // NB2
PB = DB // 2
OB = H * E // NB2
UB = 224
NA = 4
PITCH = D // 2 + 4
WO_BASE = 3 * H * PITCH + 352
WOUT_BASE = WO_BASE + KD * (H * E // 2)
W_ROWS = WOUT_BASE + KD * (FH // 2) + 16

SEM_X = 0
SEM_WIN = SEM_X + NB
SEM_GRP = SEM_WIN + len(WPIECES)
SEM_SMALL = SEM_GRP + NB2
SEM_OUT = SEM_SMALL + 1
NSEM = SEM_OUT + 1


def _slab(hd):
    return ((hd % 2) * 2 + hd // 16) * 8 + (hd % 16) // 2


def _dot(a, b):
    return lax.dot_general(a, b, (((1,), (0,)), ((), ())), preferred_element_type=F32)


def _dot_nt(a, b):
    return lax.dot_general(a, b, (((1,), (1,)), ((), ())), preferred_element_type=F32)


def _ln(x):
    m = jnp.mean(x, axis=-1, keepdims=True)
    c = x - m
    v = jnp.mean(c * c, axis=-1, keepdims=True)
    return c * lax.rsqrt(v + EPS)


def _gelu(x):
    t = jnp.tanh(x * (0.7978845608028654 + (0.7978845608028654 * 0.044715) * (x * x)))
    hx = 0.5 * x
    return hx + hx * t


def _recip(l):
    r = pl.reciprocal(l, approx=True)
    return r * (2.0 - l * r)


def _fold2(xs, f):
    a, b = xs[0], xs[1]
    for n in range(2, len(xs), 2):
        a, b = f(a, xs[n]), f(b, xs[n + 1])
    return f(a, b)


def _kernel(x_hbm, mem0_hbm, wq_hbm, wk_hbm, wv_hbm, wo_hbm, win_hbm, wsp_hbm, bsp_hbm, wout_hbm,
            out_hbm,
            x_s, xn_s, raw_s, w_u, wo_s, win_s, wsp_s, z1_s, y_s, z2_s, u_s, out_s, st_s, kv_s,
            wout_s, b32_s, mem0_s, bsp_s, sems):
    def x_copy(c):
        return pltpu.make_async_copy(x_hbm.at[pl.ds(c * RB, RB), :], x_s.at[pl.ds(c * RB, RB), :],
                                     sems.at[SEM_X + c])

    def win_copy(p):
        lo, n = WPIECES[p]
        return pltpu.make_async_copy(win_hbm.at[pl.ds(lo, n), :], win_s.at[pl.ds(lo, n), :], sems.at[SEM_WIN + p])

    def grp_copies(i):
        sem = sems.at[SEM_GRP + i]
        rows = pl.ds(i * (S // NB2), S // NB2)
        cs = [pltpu.make_async_copy(wsp_hbm.at[rows, :], wsp_s.at[rows, :], sem)]
        cs += [pltpu.make_async_copy(w_hbm.at[pl.ds(i * DB * H, DB * H), :],
                                     raw_s.at[wi, pl.ds(i * DB * H, DB * H), :], sem)
               for wi, w_hbm in enumerate((wq_hbm, wk_hbm, wv_hbm))]
        cs += [pltpu.make_async_copy(wo_hbm.at[pl.ds(i * OB, OB), :], wo_s.at[pl.ds(i * OB, OB), :], sem)]
        return cs

    small_copies = [pltpu.make_async_copy(bsp_hbm, bsp_s, sems.at[SEM_SMALL]),
                    pltpu.make_async_copy(mem0_hbm, mem0_s, sems.at[SEM_SMALL]),
                    pltpu.make_async_copy(wout_hbm, wout_s, sems.at[SEM_SMALL])]

    def out_copy(lo, n):
        return pltpu.make_async_copy(out_s.at[pl.ds(lo, n), :], out_hbm.at[pl.ds(lo, n), :], sems.at[SEM_OUT])

    x_copy(0).start()
    for p in range(len(WPIECES)):
        win_copy(p).start()
    for c in range(1, NB):
        x_copy(c).start()
    for cp in small_copies:
        cp.start()

    def ln_rows(lo, n):
        xn = _ln(x_s[pl.ds(lo, n), :].astype(F32))
        xn_s[pl.ds(lo, n), :] = xn
        return xn.astype(BF16)

    def z2_chunk(xb, t0, nt, k, lo, n):
        z = _gelu(_dot_nt(win_s[FH + lo:FH + lo + n, :], xb))
        for t in range(nt):
            y_s[t0 + t, lo:lo + n, :] = z[:, t * 128:(t + 1) * 128]
        z3 = z.reshape(n // 8, 8, nt * 128)
        st_s[0, k, :, t0 * 128:(t0 + nt) * 128] = jnp.sum(z3, axis=0)
        st_s[1, k, :, t0 * 128:(t0 + nt) * 128] = jnp.sum(z3 * z3, axis=0)

    def z1_half(c):
        xb = xn_s[pl.ds(pl.multiple_of(c * RB, RB), RB), :].astype(BF16)
        m = jnp.sum(jnp.sum(st_s[0], axis=0), axis=0, keepdims=True) * (1.0 / FH)
        s2 = jnp.sum(jnp.sum(st_s[1], axis=0), axis=0, keepdims=True) * (1.0 / FH)
        r = lax.rsqrt(jnp.maximum(s2 - m * m, 0.0) + EPS)
        mr = m * r
        pieces = [(t, hf) for t in range(TPB) for hf in range(2)]
        hf_rows = FH // 2
        for lo, n in MCH:
            z = _gelu(_dot_nt(win_s[lo:lo + n, :], xb))
            for t in range(TPB):
                z1_s[c * TPB + t, lo:lo + n, :] = z[:, t * 128:(t + 1) * 128]
                if pieces:
                    z2_s[0, FH:FH + 16, :] = z[0:16, t * 128:(t + 1) * 128].astype(BF16)
                    tp, hf = pieces.pop(0)
                    sl = slice(tp * 128, (tp + 1) * 128)
                    rows = slice(hf * hf_rows, (hf + 1) * hf_rows)
                    z2_s[c * TPB + tp, rows, :] = (y_s[tp, rows, :] * r[:, sl] - mr[:, sl]).astype(BF16)

    x_copy(0).wait()
    xb0 = ln_rows(0, RB)
    for k, (lo, n) in enumerate(MCH0):
        if k < 2:
            win_copy(k).wait()
        if k == 1:
            for cp in grp_copies(0) + grp_copies(1):
                cp.start()
        z2_chunk(xb0, 0, TPB, k, lo, n)
    win_copy(2).wait()

    def phase1_body(c, carry):
        x_copy(c + 1).wait()
        z1_half(c)
        for t in range(TPB):
            xb = ln_rows(pl.multiple_of((c + 1) * RB + t * 128, 128), 128)
            for k, (lo, n) in enumerate(MCH):
                z2_chunk(xb, t, 1, k, lo, n)
        return c + 1

    c_last = lax.fori_loop(0, NB - 1, phase1_body, 0)
    for i in range(2, NB2):
        for cp in grp_copies(i):
            cp.start()
    z1_half(c_last)
    for cp in small_copies:
        cp.wait()
    b32_s[...] = bsp_s[...].astype(F32)

    def phase2_body(i, carry):
        for cp in grp_copies(i):
            cp.wait()
        dst = w_u.at[pl.ds(pl.multiple_of(i * PB, PB), 3 * H * PITCH + PB), :]
        r_wo = pl.multiple_of(i * OB, OB)
        r_wout = pl.multiple_of(jnp.minimum(i * UB, FH - UB), 16)

        def relayout(units):
            for kind, a, b in units:
                if kind == "qkv":
                    src = raw_s.at[a, pl.ds(pl.multiple_of(i * DB * H, DB * H), DB * H), :]
                    for hi in range(2):
                        wa = pltpu.bitcast(src[pl.ds(2 * b * H + hi * 16, 16), :], U32)
                        wb = pltpu.bitcast(src[pl.ds(2 * b * H + H + hi * 16, 16), :], U32)
                        dst[pl.ds((a * H + hi * 8) * PITCH + b, 8, stride=PITCH), :] = (
                            (wa & jnp.uint32(0xFFFF)) | (wb << 16))
                        dst[pl.ds((a * H + 16 + hi * 8) * PITCH + b, 8, stride=PITCH), :] = (
                            (wa >> 16) | (wb & jnp.uint32(0xFFFF0000)))
                elif kind == "wo":
                    row = pl.multiple_of(WO_BASE + a * (H * E // 2) + b // 2 + i * (OB // 2), 8)
                    w_u[pl.ds(row, 16), :] = pltpu.bitcast(wo_s[pl.ds(r_wo + b, 32), a * 128:(a + 1) * 128], U32)
                else:
                    row = pl.multiple_of(WOUT_BASE + a * (FH // 2) + b // 2 + r_wout // 2, 8)
                    w_u[pl.ds(row, 16), :] = pltpu.bitcast(wout_s[pl.ds(r_wout + b, 32), a * 128:(a + 1) * 128], U32)

        uq = [("qkv", wi, p) for wi in range(3) for p in range(PB)]
        uo = [("wo", c, r) for c in range(KD) for r in range(0, OB, 32)]
        uo += [("wout", c, r) for c in range(KD) for r in range(0, UB, 32)]
        keyed = [(n / len(uq), u) for n, u in enumerate(uq)] + [(n / len(uo), u) for n, u in enumerate(uo)]
        units = [u for _, u in sorted(keyed, key=lambda t: t[0])]
        nslot = TPB2 * len(MCH) - 2
        per = -(-len(units) // nslot)
        slot = 0
        for t in range(TPB2):
            tt = i * TPB2 + t
            brow = b32_s[pl.ds(tt, 1), :]
            for lo, n in MCH:
                z2 = jnp.concatenate([z2_s[j, lo:lo + n, :] for j in range(NT)], axis=1)
                g = _dot_nt(z2, wsp_s[pl.ds(pl.multiple_of(tt * 128, 128), 128), :]) + brow
                z1_s[tt, lo:lo + n, :] = z1_s[tt, lo:lo + n, :] * g
                if slot < nslot:
                    mine = units[slot * per:(slot + 1) * per]
                    sub = -(-len(mine) // NA)
                    for ai in range(NA):
                        rr = n * (ai + 1) // NA
                        w_u[D // 2:D // 2 + 4, :] = pltpu.bitcast(g[rr - 8:rr - 4, :], U32)
                        relayout(mine[ai * sub:(ai + 1) * sub])
                slot += 1
        return carry

    lax.fori_loop(0, NB2, phase2_body, 0)

    scale = E ** -0.5 * LOG2E
    neg = -1e9 * LOG2E
    NV = M + 8
    qi = lax.broadcasted_iota(jnp.int32, (L - 8, L), 0)
    ki = lax.broadcasted_iota(jnp.int32, (L - 8, L), 1)
    mask = (qi < M) | (qi + 8 >= ki)
    row8 = lax.broadcasted_iota(jnp.int32, (8, 1), 0)

    def weights(starts, rows):
        return jnp.concatenate([pltpu.bitcast(w_u[s0:s0 + rows // 2, :], BF16) for s0 in starts], axis=1)

    def segment(i, j, mem):
        tile = pl.ds(pl.multiple_of(i * 128, 128), 128)
        seg = slice(j * SEG, (j + 1) * SEG)
        qkv = [None] * H
        ps = [None] * H
        ov = [None] * H
        outs = [None] * H

        def proj(hd):
            hq = h
            if hd >= SKV:
                mq = jnp.concatenate([h[:M, :E] + ov[hd - SKV] * 0.0, h[:M, E:]], axis=1)
                hq = jnp.concatenate([mq, h[M:]], axis=0)
            k, q, v = [_dot(lhs, weights([(wi * H + _slab(hd)) * PITCH], D))
                       for lhs, wi in ((h, 1), (hq, 0), (h, 2))]
            qkv[hd] = (q, k, v)

        def scores(hd):
            q, k, v = qkv[hd]
            sc = _dot_nt(jnp.concatenate([q[:M], q[NV:]], axis=0), k) * scale
            sc = jnp.where(mask, sc, neg)
            p = jnp.exp2(sc - jnp.max(sc, axis=-1, keepdims=True))
            ps[hd] = p * _recip(jnp.sum(p, axis=-1, keepdims=True))
            kv = kv_s.at[hd % KVN]
            kv[0] = k[:NV]
            kv[1] = v[:NV]
            kk = [kv[0, b:b + 4, :] for b in range(0, NV, 4)]
            vv = [kv[1, b:b + 4, :] for b in range(0, NV, 4)]
            qv = q[M:NV] * scale
            ss = []
            for n in range(NV):
                t = jnp.sum(qv * kk[n // 4][n % 4:n % 4 + 1], axis=-1, keepdims=True)
                ss.append(jnp.where(row8 >= n - M, t, neg) if n > M else t)
            mx = _fold2(ss, jnp.maximum)
            es = [jnp.exp2(t - mx) for t in ss]
            inv = _recip(_fold2(es, jnp.add))
            ov[hd] = _fold2([e * vv[n // 4][n % 4:n % 4 + 1] for n, e in enumerate(es)], jnp.add) * inv

        def pv(hd):
            p = ps[hd]
            if hd + SKV >= H:
                p = jnp.concatenate([p[:M] + ov[hd][:, :L] * 0.0, p[M:]], axis=0)
            o = _dot(p, qkv[hd][2])
            outs[hd] = jnp.concatenate([o[:M], ov[hd], o[M:]], axis=0)

        def wo(a, b):
            w = weights([WO_BASE + c * (H * E // 2) + a * E // 2 for c in range(KD)], (b - a) * E)
            return _dot(jnp.concatenate(outs[a:b], axis=1), w)

        def silu_gate():
            bo = _dot(u_s[seg, :], weights([WOUT_BASE + c * (FH // 2) for c in range(KD)], FH))
            return bo * jax.nn.sigmoid(bo)

        if j > 0:
            gate = silu_gate()
        h = jnp.concatenate([mem, xn_s.at[tile, :][seg, :]], axis=0)
        for hd in range(H):
            proj(hd)
            if hd >= SK1:
                scores(hd - SK1)
            if hd >= SK2:
                pv(hd - SK2)
        y = None
        a = 0
        for t in range(H, H + SK2):
            yp = wo(a, a + 4)
            a += 4
            y = yp if y is None else y + yp
            if t - SK1 < H:
                scores(t - SK1)
            pv(t - SK2)
        y = y + wo(a, H - 4)
        if j == 0:
            gate = silu_gate()
        y = y + wo(H - 4, H)
        out_s.at[tile, :][seg, :] = (x_s.at[tile, :][seg, :].astype(F32) + y[M:] * gate).astype(BF16)
        return y[:M]

    def phase3_body(i, mem):
        for q in range(0, FH, 128):
            w = min(128, FH - q)
            u_s[:, q:q + w] = z1_s[i, q:q + w, :].T
        for j in range(UN):
            mem = segment(i, j, mem)
            if j == UN - 2:
                out_copy(pl.multiple_of(i * 128, 128), 128 - SEG).start()
        out_copy(pl.multiple_of(i * 128 + 128 - SEG, SEG), SEG).start()
        return mem

    lax.fori_loop(0, NT, phase3_body, mem0_s[...].astype(F32))
    out_copy(0, S).wait()


def pallas_recurrent_scan__memory_aug_recurrent_mem_tr__mixer_gmlp__prompt_kernel(
    A_x, A_mem0, A_Wq, A_Wk, A_Wv, A_Wo, A_seg_len, B_x, B_w_in, B_w_sp, B_b_sp, B_w_out,
):
    assert A_x.shape == (1, S, D) and A_Wq.shape == (D, H, E) and B_w_in.shape == (D, 2 * FH)
    if isinstance(A_seg_len, int):
        assert A_seg_len == SEG
    hbm = pl.BlockSpec(memory_space=pl.ANY)
    out = pl.pallas_call(
        _kernel,
        out_shape=jax.ShapeDtypeStruct((S, D), BF16),
        in_specs=[hbm] * 10,
        out_specs=hbm,
        scratch_shapes=[
            pltpu.VMEM((S, D), BF16),
            pltpu.VMEM((S, D), F32),
            pltpu.VMEM((3, D * H, E), BF16),
            pltpu.VMEM((W_ROWS, E), U32),
            pltpu.VMEM((H * E, D), BF16),
            pltpu.VMEM((2 * FH, D), BF16),
            pltpu.VMEM((S, S), BF16),
            pltpu.VMEM((NT, FH, 128), F32),
            pltpu.VMEM((TPB, FH, 128), F32),
            pltpu.VMEM((NT, FH + 32, 128), BF16),
            pltpu.VMEM((128, FH), F32),
            pltpu.VMEM((S, D), BF16),
            pltpu.VMEM((2, len(MCH), 8, RB), F32),
            pltpu.VMEM((KVN, 2, M + 8, E), F32),
            pltpu.VMEM((FH, D), BF16),
            pltpu.VMEM((NT, 128), F32),
            pltpu.VMEM((M, D), BF16),
            pltpu.VMEM((NT, 128), BF16),
            pltpu.SemaphoreType.DMA((NSEM,)),
        ],
        compiler_params=pltpu.CompilerParams(vmem_limit_bytes=120 * 1024 * 1024),
    )(A_x.reshape(S, D), A_mem0.reshape(M, D), A_Wq.reshape(D * H, E), A_Wk.reshape(D * H, E),
      A_Wv.reshape(D * H, E), A_Wo.reshape(H * E, D), B_w_in.T, B_w_sp, B_b_sp.reshape(NT, 128), B_w_out)
    return out.reshape(1, S, D)
```

```python
import jax
import jax.numpy as jnp
from jax import lax
import jax.experimental.pallas as pl
import jax.experimental.pallas.tpu as pltpu

F32 = jnp.float32
BF16 = jnp.bfloat16
U32 = jnp.uint32

S, D, H, E, M, SEG = 2048, 640, 32, 128, 8, 32
L = M + SEG
FH = 864
EPS = 1e-5
LOG2E = 1.4426950408889634

SK1 = 2
SK2 = 6
SKV = 5
KVN = 16
UN = 128 // SEG
NT = S // 128
KD = D // 128

NB = 4
RB = S // NB
TPB = RB // 128
MCH = [(0, 256), (256, 256), (512, 256), (768, 96)]
MCH0 = [(0, 288), (288, 192), (480, 192), (672, 192)]
WPIECES = [(FH, 288), (FH + 288, FH - 288), (0, FH)]

NB2 = 4
TPB2 = NT // NB2
DB = D // NB2
PB = DB // 2
OB = H * E // NB2
UB = 224
NA = 4
PITCH = D // 2 + 4
WO_BASE = 3 * H * PITCH + 352
WOUT_BASE = WO_BASE + KD * (H * E // 2)
W_ROWS = WOUT_BASE + KD * (FH // 2) + 16

SEM_X = 0
SEM_WIN = SEM_X + NB
SEM_GRP = SEM_WIN + len(WPIECES)
SEM_SMALL = SEM_GRP + NB2
SEM_OUT = SEM_SMALL + 1
NSEM = SEM_OUT + 1


def _slab(hd):
    return ((hd % 2) * 2 + hd // 16) * 8 + (hd % 16) // 2


def _dot(a, b):
    return lax.dot_general(a, b, (((1,), (0,)), ((), ())), preferred_element_type=F32)


def _dot_nt(a, b):
    return lax.dot_general(a, b, (((1,), (1,)), ((), ())), preferred_element_type=F32)


def _ln(x):
    m = jnp.mean(x, axis=-1, keepdims=True)
    c = x - m
    v = jnp.mean(c * c, axis=-1, keepdims=True)
    return c * lax.rsqrt(v + EPS)


def _gelu(x):
    t = jnp.tanh(x * (0.7978845608028654 + (0.7978845608028654 * 0.044715) * (x * x)))
    hx = 0.5 * x
    return hx + hx * t


def _recip(l):
    r = pl.reciprocal(l, approx=True)
    return r * (2.0 - l * r)


def _fold2(xs, f):
    a, b = xs[0], xs[1]
    for n in range(2, len(xs), 2):
        a, b = f(a, xs[n]), f(b, xs[n + 1])
    return f(a, b)


def _kernel(x_hbm, mem0_hbm, wq_hbm, wk_hbm, wv_hbm, wo_hbm, win_hbm, wsp_hbm, bsp_hbm, wout_hbm,
            out_hbm,
            x_s, xn_s, raw_s, w_u, wo_s, win_s, wsp_s, z1_s, y_s, z2_s, u_s, out_s, st_s, kv_s,
            wout_s, b32_s, mem0_s, bsp_s, sems):
    def x_copy(c):
        return pltpu.make_async_copy(x_hbm.at[pl.ds(c * RB, RB), :], x_s.at[pl.ds(c * RB, RB), :],
                                     sems.at[SEM_X + c])

    def win_copy(p):
        lo, n = WPIECES[p]
        return pltpu.make_async_copy(win_hbm.at[pl.ds(lo, n), :], win_s.at[pl.ds(lo, n), :], sems.at[SEM_WIN + p])

    def grp_copies(i):
        sem = sems.at[SEM_GRP + i]
        rows = pl.ds(i * (S // NB2), S // NB2)
        cs = [pltpu.make_async_copy(wsp_hbm.at[rows, :], wsp_s.at[rows, :], sem)]
        cs += [pltpu.make_async_copy(w_hbm.at[pl.ds(i * DB * H, DB * H), :],
                                     raw_s.at[wi, pl.ds(i * DB * H, DB * H), :], sem)
               for wi, w_hbm in enumerate((wq_hbm, wk_hbm, wv_hbm))]
        cs += [pltpu.make_async_copy(wo_hbm.at[pl.ds(i * OB, OB), :], wo_s.at[pl.ds(i * OB, OB), :], sem)]
        return cs

    small_copies = [pltpu.make_async_copy(bsp_hbm, bsp_s, sems.at[SEM_SMALL]),
                    pltpu.make_async_copy(mem0_hbm, mem0_s, sems.at[SEM_SMALL]),
                    pltpu.make_async_copy(wout_hbm, wout_s, sems.at[SEM_SMALL])]

    def out_copy(lo, n):
        return pltpu.make_async_copy(out_s.at[pl.ds(lo, n), :], out_hbm.at[pl.ds(lo, n), :], sems.at[SEM_OUT])

    x_copy(0).start()
    for p in range(len(WPIECES)):
        win_copy(p).start()
    for c in range(1, NB):
        x_copy(c).start()
    for cp in small_copies:
        cp.start()

    def ln_rows(lo, n):
        xn = _ln(x_s[pl.ds(lo, n), :].astype(F32))
        xn_s[pl.ds(lo, n), :] = xn
        return xn.astype(BF16)

    def z2_chunk(xb, t0, nt, k, lo, n):
        z = _gelu(_dot_nt(win_s[FH + lo:FH + lo + n, :], xb))
        for t in range(nt):
            y_s[t0 + t, lo:lo + n, :] = z[:, t * 128:(t + 1) * 128]
        z3 = z.reshape(n // 8, 8, nt * 128)
        st_s[0, k, :, t0 * 128:(t0 + nt) * 128] = jnp.sum(z3, axis=0)
        st_s[1, k, :, t0 * 128:(t0 + nt) * 128] = jnp.sum(z3 * z3, axis=0)

    def z1_half(c):
        xb = xn_s[pl.ds(pl.multiple_of(c * RB, RB), RB), :].astype(BF16)
        m = jnp.sum(jnp.sum(st_s[0], axis=0), axis=0, keepdims=True) * (1.0 / FH)
        s2 = jnp.sum(jnp.sum(st_s[1], axis=0), axis=0, keepdims=True) * (1.0 / FH)
        r = lax.rsqrt(jnp.maximum(s2 - m * m, 0.0) + EPS)
        mr = m * r
        pieces = [(t, hf) for t in range(TPB) for hf in range(2)]
        hf_rows = FH // 2
        for lo, n in MCH:
            z = _gelu(_dot_nt(win_s[lo:lo + n, :], xb))
            for t in range(TPB):
                z1_s[c * TPB + t, lo:lo + n, :] = z[:, t * 128:(t + 1) * 128]
                if pieces:
                    z2_s[0, FH:FH + 16, :] = z[0:16, t * 128:(t + 1) * 128].astype(BF16)
                    tp, hf = pieces.pop(0)
                    sl = slice(tp * 128, (tp + 1) * 128)
                    rows = slice(hf * hf_rows, (hf + 1) * hf_rows)
                    z2_s[c * TPB + tp, rows, :] = (y_s[tp, rows, :] * r[:, sl] - mr[:, sl]).astype(BF16)

    x_copy(0).wait()
    xb0 = ln_rows(0, RB)
    for k, (lo, n) in enumerate(MCH0):
        if k < 2:
            win_copy(k).wait()
        if k == 1:
            for cp in grp_copies(0) + grp_copies(1):
                cp.start()
        z2_chunk(xb0, 0, TPB, k, lo, n)
    win_copy(2).wait()

    def phase1_body(c, carry):
        x_copy(c + 1).wait()
        z1_half(c)
        for t in range(TPB):
            xb = ln_rows(pl.multiple_of((c + 1) * RB + t * 128, 128), 128)
            for k, (lo, n) in enumerate(MCH):
                z2_chunk(xb, t, 1, k, lo, n)
        return c + 1

    c_last = lax.fori_loop(0, NB - 1, phase1_body, 0)
    for i in range(2, NB2):
        for cp in grp_copies(i):
            cp.start()
    z1_half(c_last)
    for cp in small_copies:
        cp.wait()
    b32_s[...] = bsp_s[...].astype(F32)

    def phase2_body(i, carry):
        for cp in grp_copies(i):
            cp.wait()
        dst = w_u.at[pl.ds(pl.multiple_of(i * PB, PB), 3 * H * PITCH + PB), :]
        r_wout = pl.multiple_of(jnp.minimum(i * UB, FH - UB), 32)
        wo_src = wo_s.at[pl.ds(pl.multiple_of(i * OB, OB), OB), :]
        wo_dst = w_u.at[pl.ds(pl.multiple_of(WO_BASE + i * (OB // 2), 32), (KD - 1) * (H * E // 2) + OB // 2), :]
        wout_src = wout_s.at[pl.ds(r_wout, UB), :]
        wout_dst = w_u.at[pl.ds(pl.multiple_of(WOUT_BASE + r_wout // 2, 16), (KD - 1) * (FH // 2) + UB // 2), :]

        def relayout(units):
            for kind, a, b in units:
                if kind == "qkv":
                    src = raw_s.at[a, pl.ds(pl.multiple_of(i * DB * H, DB * H), DB * H), :]
                    for hi in range(2):
                        wa = pltpu.bitcast(src[pl.ds(2 * b * H + hi * 16, 16), :], U32)
                        wb = pltpu.bitcast(src[pl.ds(2 * b * H + H + hi * 16, 16), :], U32)
                        dst[pl.ds((a * H + hi * 8) * PITCH + b, 8, stride=PITCH), :] = (
                            (wa & jnp.uint32(0xFFFF)) | (wb << 16))
                        dst[pl.ds((a * H + 16 + hi * 8) * PITCH + b, 8, stride=PITCH), :] = (
                            (wa >> 16) | (wb & jnp.uint32(0xFFFF0000)))
                elif kind == "wo":
                    wo_dst[pl.ds(a * (H * E // 2) + b // 2, 16), :] = (
                        pltpu.bitcast(wo_src[b:b + 32, a * 128:(a + 1) * 128], U32))
                else:
                    wout_dst[pl.ds(a * (FH // 2) + b // 2, 16), :] = (
                        pltpu.bitcast(wout_src[b:b + 32, a * 128:(a + 1) * 128], U32))

        uq = [("qkv", wi, p) for wi in range(3) for p in range(PB)]
        uo = [("wo", c, r) for c in range(KD) for r in range(0, OB, 32)]
        uo += [("wout", c, r) for c in range(KD) for r in range(0, UB, 32)]
        keyed = [(n / len(uq), u) for n, u in enumerate(uq)] + [(n / len(uo), u) for n, u in enumerate(uo)]
        units = [u for _, u in sorted(keyed, key=lambda t: t[0])]
        nslot = TPB2 * len(MCH) - 2
        per = -(-len(units) // nslot)
        slot = 0
        for t in range(TPB2):
            tt = i * TPB2 + t
            brow = b32_s[pl.ds(tt, 1), :]
            for lo, n in MCH:
                z2 = jnp.concatenate([z2_s[j, lo:lo + n, :] for j in range(NT)], axis=1)
                g = _dot_nt(z2, wsp_s[pl.ds(pl.multiple_of(tt * 128, 128), 128), :]) + brow
                z1_s[tt, lo:lo + n, :] = z1_s[tt, lo:lo + n, :] * g
                if slot < nslot:
                    mine = units[slot * per:(slot + 1) * per]
                    sub = -(-len(mine) // NA)
                    for ai in range(NA):
                        rr = n * (ai + 1) // NA
                        w_u[D // 2:D // 2 + 4, :] = pltpu.bitcast(g[rr - 8:rr - 4, :], U32)
                        relayout(mine[ai * sub:(ai + 1) * sub])
                slot += 1
        return carry

    lax.fori_loop(0, NB2, phase2_body, 0)

    scale = E ** -0.5 * LOG2E
    neg = -1e9 * LOG2E
    NV = M + 8
    qi = lax.broadcasted_iota(jnp.int32, (L - 8, L), 0)
    ki = lax.broadcasted_iota(jnp.int32, (L - 8, L), 1)
    mask = (qi < M) | (qi + 8 >= ki)
    row8 = lax.broadcasted_iota(jnp.int32, (8, 1), 0)

    def weights(starts, rows):
        return jnp.concatenate([pltpu.bitcast(w_u[s0:s0 + rows // 2, :], BF16) for s0 in starts], axis=1)

    def segment(i, j, mem):
        tile = pl.ds(pl.multiple_of(i * 128, 128), 128)
        seg = slice(j * SEG, (j + 1) * SEG)
        qkv = [None] * H
        ps = [None] * H
        ov = [None] * H
        outs = [None] * H

        def proj(hd):
            hq = h
            if hd >= SKV:
                mq = jnp.concatenate([h[:M, :E] + ov[hd - SKV] * 0.0, h[:M, E:]], axis=1)
                hq = jnp.concatenate([mq, h[M:]], axis=0)
            k, q, v = [_dot(lhs, weights([(wi * H + _slab(hd)) * PITCH], D))
                       for lhs, wi in ((h, 1), (hq, 0), (h, 2))]
            qkv[hd] = (q, k, v)

        def scores(hd):
            q, k, v = qkv[hd]
            sc = _dot_nt(jnp.concatenate([q[:M], q[NV:]], axis=0), k) * scale
            sc = jnp.where(mask, sc, neg)
            p = jnp.exp2(sc - jnp.max(sc, axis=-1, keepdims=True))
            ps[hd] = p * _recip(jnp.sum(p, axis=-1, keepdims=True))
            kv = kv_s.at[hd % KVN]
            kv[0] = k[:NV]
            kv[1] = v[:NV]
            kk = [kv[0, b:b + 4, :] for b in range(0, NV, 4)]
            vv = [kv[1, b:b + 4, :] for b in range(0, NV, 4)]
            qv = q[M:NV] * scale
            ss = []
            for n in range(NV):
                t = jnp.sum(qv * kk[n // 4][n % 4:n % 4 + 1], axis=-1, keepdims=True)
                ss.append(jnp.where(row8 >= n - M, t, neg) if n > M else t)
            mx = _fold2(ss, jnp.maximum)
            es = [jnp.exp2(t - mx) for t in ss]
            inv = _recip(_fold2(es, jnp.add))
            ov[hd] = _fold2([e * vv[n // 4][n % 4:n % 4 + 1] for n, e in enumerate(es)], jnp.add) * inv

        def pv(hd):
            p = ps[hd]
            if hd + SKV >= H:
                p = jnp.concatenate([p[:M] + ov[hd][:, :L] * 0.0, p[M:]], axis=0)
            o = _dot(p, qkv[hd][2])
            outs[hd] = jnp.concatenate([o[:M], ov[hd], o[M:]], axis=0)

        def wo(a, b):
            w = weights([WO_BASE + c * (H * E // 2) + a * E // 2 for c in range(KD)], (b - a) * E)
            return _dot(jnp.concatenate(outs[a:b], axis=1), w)

        def silu_gate():
            bo = _dot(u_s[seg, :], weights([WOUT_BASE + c * (FH // 2) for c in range(KD)], FH))
            return bo * jax.nn.sigmoid(bo)

        if j > 0:
            gate = silu_gate()
        h = jnp.concatenate([mem, xn_s.at[tile, :][seg, :]], axis=0)
        for hd in range(H):
            proj(hd)
            if hd >= SK1:
                scores(hd - SK1)
            if hd >= SK2:
                pv(hd - SK2)
        y = None
        a = 0
        for t in range(H, H + SK2):
            yp = wo(a, a + 4)
            a += 4
            y = yp if y is None else y + yp
            if t - SK1 < H:
                scores(t - SK1)
            pv(t - SK2)
        y = y + wo(a, H - 4)
        if j == 0:
            gate = silu_gate()
        y = y + wo(H - 4, H)
        out_s.at[tile, :][seg, :] = (x_s.at[tile, :][seg, :].astype(F32) + y[M:] * gate).astype(BF16)
        return y[:M]

    def phase3_body(i, mem):
        for q in range(0, FH, 128):
            w = min(128, FH - q)
            u_s[:, q:q + w] = z1_s[i, q:q + w, :].T
        for j in range(UN):
            mem = segment(i, j, mem)
            if j == UN - 2:
                out_copy(pl.multiple_of(i * 128, 128), 128 - SEG).start()
        out_copy(pl.multiple_of(i * 128 + 128 - SEG, SEG), SEG).start()
        return mem

    lax.fori_loop(0, NT, phase3_body, mem0_s[...].astype(F32))
    out_copy(0, S).wait()


def pallas_recurrent_scan__memory_aug_recurrent_mem_tr__mixer_gmlp__prompt_kernel(
    A_x, A_mem0, A_Wq, A_Wk, A_Wv, A_Wo, A_seg_len, B_x, B_w_in, B_w_sp, B_b_sp, B_w_out,
):
    assert A_x.shape == (1, S, D) and A_Wq.shape == (D, H, E) and B_w_in.shape == (D, 2 * FH)
    if isinstance(A_seg_len, int):
        assert A_seg_len == SEG
    hbm = pl.BlockSpec(memory_space=pl.ANY)
    out = pl.pallas_call(
        _kernel,
        out_shape=jax.ShapeDtypeStruct((S, D), BF16),
        in_specs=[hbm] * 10,
        out_specs=hbm,
        scratch_shapes=[
            pltpu.VMEM((S, D), BF16),
            pltpu.VMEM((S, D), F32),
            pltpu.VMEM((3, D * H, E), BF16),
            pltpu.VMEM((W_ROWS, E), U32),
            pltpu.VMEM((H * E, D), BF16),
            pltpu.VMEM((2 * FH, D), BF16),
            pltpu.VMEM((S, S), BF16),
            pltpu.VMEM((NT, FH, 128), F32),
            pltpu.VMEM((TPB, FH, 128), F32),
            pltpu.VMEM((NT, FH + 32, 128), BF16),
            pltpu.VMEM((128, FH), F32),
            pltpu.VMEM((S, D), BF16),
            pltpu.VMEM((2, len(MCH), 8, RB), F32),
            pltpu.VMEM((KVN, 2, M + 8, E), F32),
            pltpu.VMEM((FH, D), BF16),
            pltpu.VMEM((NT, 128), F32),
            pltpu.VMEM((M, D), BF16),
            pltpu.VMEM((NT, 128), BF16),
            pltpu.SemaphoreType.DMA((NSEM,)),
        ],
        compiler_params=pltpu.CompilerParams(vmem_limit_bytes=120 * 1024 * 1024),
    )(A_x.reshape(S, D), A_mem0.reshape(M, D), A_Wq.reshape(D * H, E), A_Wk.reshape(D * H, E),
      A_Wv.reshape(D * H, E), A_Wo.reshape(H * E, D), B_w_in.T, B_w_sp, B_b_sp.reshape(NT, 128), B_w_out)
    return out.reshape(1, S, D)
```

```python
import jax
import jax.numpy as jnp
from jax import lax
import jax.experimental.pallas as pl
import jax.experimental.pallas.tpu as pltpu

F32 = jnp.float32
BF16 = jnp.bfloat16
U32 = jnp.uint32

S, D, H, E, M, SEG = 2048, 640, 32, 128, 8, 32
L = M + SEG
FH = 864
EPS = 1e-5
LOG2E = 1.4426950408889634

SK1 = 2
SK2 = 6
SKV = 5
KVN = 8
UN = 128 // SEG
NT = S // 128
KD = D // 128

NB = 4
RB = S // NB
TPB = RB // 128
MCH = [(0, 256), (256, 256), (512, 256), (768, 96)]
MCH0 = [(0, 288), (288, 192), (480, 192), (672, 192)]
WPIECES = [(FH, 288), (FH + 288, FH - 288), (0, FH)]

NB2 = 4
TPB2 = NT // NB2
DB = D // NB2
PB = DB // 2
OB = H * E // NB2
UB = 224
NA = 4
PITCH = D // 2 + 4
WO_BASE = 3 * H * PITCH + 352
WOUT_BASE = WO_BASE + KD * (H * E // 2)
W_ROWS = WOUT_BASE + KD * (FH // 2) + 16

SEM_X = 0
SEM_WIN = SEM_X + NB
SEM_GRP = SEM_WIN + len(WPIECES)
SEM_SMALL = SEM_GRP + NB2
SEM_OUT = SEM_SMALL + 1
NSEM = SEM_OUT + 1


def _slab(hd):
    return ((hd % 2) * 2 + hd // 16) * 8 + (hd % 16) // 2


def _dot(a, b):
    return lax.dot_general(a, b, (((1,), (0,)), ((), ())), preferred_element_type=F32)


def _dot_nt(a, b):
    return lax.dot_general(a, b, (((1,), (1,)), ((), ())), preferred_element_type=F32)


def _ln(x):
    m = jnp.mean(x, axis=-1, keepdims=True)
    c = x - m
    v = jnp.mean(c * c, axis=-1, keepdims=True)
    return c * lax.rsqrt(v + EPS)


def _gelu(x):
    t = jnp.tanh(x * (0.7978845608028654 + (0.7978845608028654 * 0.044715) * (x * x)))
    hx = 0.5 * x
    return hx + hx * t


def _recip(l):
    r = pl.reciprocal(l, approx=True)
    return r * (2.0 - l * r)


def _fold2(xs, f):
    a, b = xs[0], xs[1]
    for n in range(2, len(xs), 2):
        a, b = f(a, xs[n]), f(b, xs[n + 1])
    return f(a, b)


def _kernel(x_hbm, mem0_hbm, wq_hbm, wk_hbm, wv_hbm, wo_hbm, win_hbm, wsp_hbm, bsp_hbm, wout_hbm,
            out_hbm,
            x_s, xn_s, raw_s, w_u, wo_s, win_s, wsp_s, z1_s, y_s, z2_s, u_s, out_s, st_s, kv_s,
            wout_s, b32_s, mem0_s, bsp_s, sems):
    def x_copy(c):
        return pltpu.make_async_copy(x_hbm.at[pl.ds(c * RB, RB), :], x_s.at[pl.ds(c * RB, RB), :],
                                     sems.at[SEM_X + c])

    def win_copy(p):
        lo, n = WPIECES[p]
        return pltpu.make_async_copy(win_hbm.at[pl.ds(lo, n), :], win_s.at[pl.ds(lo, n), :], sems.at[SEM_WIN + p])

    def grp_copies(i):
        sem = sems.at[SEM_GRP + i]
        rows = pl.ds(i * (S // NB2), S // NB2)
        cs = [pltpu.make_async_copy(wsp_hbm.at[rows, :], wsp_s.at[rows, :], sem)]
        cs += [pltpu.make_async_copy(w_hbm.at[pl.ds(i * DB * H, DB * H), :],
                                     raw_s.at[wi, pl.ds(i * DB * H, DB * H), :], sem)
               for wi, w_hbm in enumerate((wq_hbm, wk_hbm, wv_hbm))]
        cs += [pltpu.make_async_copy(wo_hbm.at[pl.ds(i * OB, OB), :], wo_s.at[pl.ds(i * OB, OB), :], sem)]
        return cs

    small_copies = [pltpu.make_async_copy(bsp_hbm, bsp_s, sems.at[SEM_SMALL]),
                    pltpu.make_async_copy(mem0_hbm, mem0_s, sems.at[SEM_SMALL]),
                    pltpu.make_async_copy(wout_hbm, wout_s, sems.at[SEM_SMALL])]

    def out_copy(lo, n):
        return pltpu.make_async_copy(out_s.at[pl.ds(lo, n), :], out_hbm.at[pl.ds(lo, n), :], sems.at[SEM_OUT])

    x_copy(0).start()
    for p in range(len(WPIECES)):
        win_copy(p).start()
    for c in range(1, NB):
        x_copy(c).start()
    for cp in small_copies:
        cp.start()

    def ln_rows(lo, n):
        xn = _ln(x_s[pl.ds(lo, n), :].astype(F32))
        xn_s[pl.ds(lo, n), :] = xn
        return xn.astype(BF16)

    def z2_chunk(xb, t0, nt, k, lo, n):
        z = _gelu(_dot_nt(win_s[FH + lo:FH + lo + n, :], xb))
        for t in range(nt):
            y_s[t0 + t, lo:lo + n, :] = z[:, t * 128:(t + 1) * 128]
        z3 = z.reshape(n // 8, 8, nt * 128)
        st_s[0, k, :, t0 * 128:(t0 + nt) * 128] = jnp.sum(z3, axis=0)
        st_s[1, k, :, t0 * 128:(t0 + nt) * 128] = jnp.sum(z3 * z3, axis=0)

    def z1_half(c):
        xb = xn_s[pl.ds(pl.multiple_of(c * RB, RB), RB), :].astype(BF16)
        m = jnp.sum(jnp.sum(st_s[0], axis=0), axis=0, keepdims=True) * (1.0 / FH)
        s2 = jnp.sum(jnp.sum(st_s[1], axis=0), axis=0, keepdims=True) * (1.0 / FH)
        r = lax.rsqrt(jnp.maximum(s2 - m * m, 0.0) + EPS)
        mr = m * r
        pieces = [(t, hf) for t in range(TPB) for hf in range(2)]
        hf_rows = FH // 2
        for lo, n in MCH:
            z = _gelu(_dot_nt(win_s[lo:lo + n, :], xb))
            for t in range(TPB):
                z1_s[c * TPB + t, lo:lo + n, :] = z[:, t * 128:(t + 1) * 128]
                if pieces:
                    z2_s[0, FH:FH + 16, :] = z[0:16, t * 128:(t + 1) * 128].astype(BF16)
                    tp, hf = pieces.pop(0)
                    sl = slice(tp * 128, (tp + 1) * 128)
                    rows = slice(hf * hf_rows, (hf + 1) * hf_rows)
                    z2_s[c * TPB + tp, rows, :] = (y_s[tp, rows, :] * r[:, sl] - mr[:, sl]).astype(BF16)

    x_copy(0).wait()
    xb0 = ln_rows(0, RB)
    for k, (lo, n) in enumerate(MCH0):
        if k < 2:
            win_copy(k).wait()
        if k == 1:
            for cp in grp_copies(0) + grp_copies(1):
                cp.start()
        z2_chunk(xb0, 0, TPB, k, lo, n)
    win_copy(2).wait()

    def phase1_body(c, carry):
        x_copy(c + 1).wait()
        z1_half(c)
        for t in range(TPB):
            xb = ln_rows(pl.multiple_of((c + 1) * RB + t * 128, 128), 128)
            for k, (lo, n) in enumerate(MCH):
                z2_chunk(xb, t, 1, k, lo, n)
        return c + 1

    c_last = lax.fori_loop(0, NB - 1, phase1_body, 0)
    for i in range(2, NB2):
        for cp in grp_copies(i):
            cp.start()
    z1_half(c_last)
    for cp in small_copies:
        cp.wait()
    b32_s[...] = bsp_s[...].astype(F32)

    def phase2_body(i, carry):
        for cp in grp_copies(i):
            cp.wait()
        dst = w_u.at[pl.ds(pl.multiple_of(i * PB, PB), 3 * H * PITCH + PB), :]
        r_wout = pl.multiple_of(jnp.minimum(i * UB, FH - UB), 32)
        wo_src = wo_s.at[pl.ds(pl.multiple_of(i * OB, OB), OB), :]
        wo_dst = w_u.at[pl.ds(pl.multiple_of(WO_BASE + i * (OB // 2), 32), (KD - 1) * (H * E // 2) + OB // 2), :]
        wout_src = wout_s.at[pl.ds(r_wout, UB), :]
        wout_dst = w_u.at[pl.ds(pl.multiple_of(WOUT_BASE + r_wout // 2, 16), (KD - 1) * (FH // 2) + UB // 2), :]

        def relayout(units):
            for kind, a, b in units:
                if kind == "qkv":
                    src = raw_s.at[a, pl.ds(pl.multiple_of(i * DB * H, DB * H), DB * H), :]
                    for hi in range(2):
                        wa = pltpu.bitcast(src[pl.ds(2 * b * H + hi * 16, 16), :], U32)
                        wb = pltpu.bitcast(src[pl.ds(2 * b * H + H + hi * 16, 16), :], U32)
                        dst[pl.ds((a * H + hi * 8) * PITCH + b, 8, stride=PITCH), :] = (
                            (wa & jnp.uint32(0xFFFF)) | (wb << 16))
                        dst[pl.ds((a * H + 16 + hi * 8) * PITCH + b, 8, stride=PITCH), :] = (
                            (wa >> 16) | (wb & jnp.uint32(0xFFFF0000)))
                elif kind == "wo":
                    wo_dst[pl.ds(a * (H * E // 2) + b // 2, 16), :] = (
                        pltpu.bitcast(wo_src[b:b + 32, a * 128:(a + 1) * 128], U32))
                else:
                    wout_dst[pl.ds(a * (FH // 2) + b // 2, 16), :] = (
                        pltpu.bitcast(wout_src[b:b + 32, a * 128:(a + 1) * 128], U32))

        uq = [("qkv", wi, p) for wi in range(3) for p in range(PB)]
        uo = [("wo", c, r) for c in range(KD) for r in range(0, OB, 32)]
        uo += [("wout", c, r) for c in range(KD) for r in range(0, UB, 32)]
        keyed = [(n / len(uq), u) for n, u in enumerate(uq)] + [(n / len(uo), u) for n, u in enumerate(uo)]
        units = [u for _, u in sorted(keyed, key=lambda t: t[0])]
        nslot = TPB2 * len(MCH) - 2
        per = -(-len(units) // nslot)
        slot = 0
        for t in range(TPB2):
            tt = i * TPB2 + t
            brow = b32_s[pl.ds(tt, 1), :]
            for lo, n in MCH:
                z2 = jnp.concatenate([z2_s[j, lo:lo + n, :] for j in range(NT)], axis=1)
                g = _dot_nt(z2, wsp_s[pl.ds(pl.multiple_of(tt * 128, 128), 128), :]) + brow
                z1_s[tt, lo:lo + n, :] = z1_s[tt, lo:lo + n, :] * g
                if slot < nslot:
                    mine = units[slot * per:(slot + 1) * per]
                    sub = -(-len(mine) // NA)
                    for ai in range(NA):
                        rr = n * (ai + 1) // NA
                        w_u[D // 2:D // 2 + 4, :] = pltpu.bitcast(g[rr - 8:rr - 4, :], U32)
                        relayout(mine[ai * sub:(ai + 1) * sub])
                slot += 1
        return carry

    lax.fori_loop(0, NB2, phase2_body, 0)

    scale = E ** -0.5 * LOG2E
    neg = -1e9 * LOG2E
    NV = M + 8
    qi = lax.broadcasted_iota(jnp.int32, (L - 8, L), 0)
    ki = lax.broadcasted_iota(jnp.int32, (L - 8, L), 1)
    mask = (qi < M) | (qi + 8 >= ki)
    row8 = lax.broadcasted_iota(jnp.int32, (8, 1), 0)

    def weights(starts, rows):
        return jnp.concatenate([pltpu.bitcast(w_u[s0:s0 + rows // 2, :], BF16) for s0 in starts], axis=1)

    def segment(i, j, mem):
        tile = pl.ds(pl.multiple_of(i * 128, 128), 128)
        seg = slice(j * SEG, (j + 1) * SEG)
        qkv = [None] * H
        ps = [None] * H
        ov = [None] * H
        outs = [None] * H

        def proj(hd):
            hk = h
            if hd >= SKV:
                mk = [h[:M, :3 * E], h[:M, 3 * E:4 * E] + ov[hd - SKV] * 0.0, h[:M, 4 * E:]]
                hk = jnp.concatenate([jnp.concatenate(mk, axis=1), h[M:]], axis=0)
            k, q, v = [_dot(lhs, weights([(wi * H + _slab(hd)) * PITCH], D))
                       for lhs, wi in ((hk, 1), (h, 0), (h, 2))]
            qkv[hd] = (q, k, v)

        def scores(hd):
            q, k, v = qkv[hd]
            sc = _dot_nt(jnp.concatenate([q[:M], q[NV:]], axis=0), k) * scale
            sc = jnp.where(mask, sc, neg)
            p = jnp.exp2(sc - jnp.max(sc, axis=-1, keepdims=True))
            ps[hd] = p * _recip(jnp.sum(p, axis=-1, keepdims=True))
            kv = kv_s.at[hd % KVN]
            kv[0] = k[:NV]
            kv[1] = v[:NV]
            kk = [kv[0, b:b + 4, :] for b in range(0, NV, 4)]
            vv = [kv[1, b:b + 4, :] for b in range(0, NV, 4)]
            qv = q[M:NV] * scale
            ss = []
            for n in range(NV):
                t = jnp.sum(qv * kk[n // 4][n % 4:n % 4 + 1], axis=-1, keepdims=True)
                ss.append(jnp.where(row8 >= n - M, t, neg) if n > M else t)
            mx = _fold2(ss, jnp.maximum)
            es = [jnp.exp2(t - mx) for t in ss]
            inv = _recip(_fold2(es, jnp.add))
            ov[hd] = _fold2([e * vv[n // 4][n % 4:n % 4 + 1] for n, e in enumerate(es)], jnp.add) * inv

        def pv(hd):
            p = ps[hd]
            if hd + SKV >= H:
                p = jnp.concatenate([p[:M] + ov[hd][:, :L] * 0.0, p[M:]], axis=0)
            o = _dot(p, qkv[hd][2])
            outs[hd] = jnp.concatenate([o[:M], ov[hd], o[M:]], axis=0)

        def wo(a, b):
            w = weights([WO_BASE + c * (H * E // 2) + a * E // 2 for c in range(KD)], (b - a) * E)
            return _dot(jnp.concatenate(outs[a:b], axis=1), w)

        def silu_gate():
            bo = _dot(u_s[seg, :], weights([WOUT_BASE + c * (FH // 2) for c in range(KD)], FH))
            return bo * jax.nn.sigmoid(bo)

        if j > 0:
            gate = silu_gate()
        h = jnp.concatenate([mem, xn_s.at[tile, :][seg, :]], axis=0)
        for hd in range(H):
            proj(hd)
            if hd >= SK1:
                scores(hd - SK1)
            if hd >= SK2:
                pv(hd - SK2)
        y = None
        a = 0
        for t in range(H, H + SK2):
            yp = wo(a, a + 4)
            a += 4
            y = yp if y is None else y + yp
            if t - SK1 < H:
                scores(t - SK1)
            pv(t - SK2)
        y = y + wo(a, H - 4)
        if j == 0:
            gate = silu_gate()
        y = y + wo(H - 4, H)
        out_s[pl.ds(pl.multiple_of(i * 128 + j * SEG, SEG), SEG), :] = (
            x_s.at[tile, :][seg, :].astype(F32) + y[M:] * gate).astype(BF16)
        return y[:M]

    def phase3_body(i, mem):
        for q in range(0, FH, 128):
            w = min(128, FH - q)
            u_s[:, q:q + w] = z1_s[i, q:q + w, :].T
        for j in range(UN):
            mem = segment(i, j, mem)
            if j == UN - 2:
                out_copy(pl.multiple_of(i * 128, 128), 128 - SEG).start()
        out_copy(pl.multiple_of(i * 128 + 128 - SEG, SEG), SEG).start()
        return mem

    lax.fori_loop(0, NT, phase3_body, mem0_s[...].astype(F32))
    out_copy(0, S).wait()


def pallas_recurrent_scan__memory_aug_recurrent_mem_tr__mixer_gmlp__prompt_kernel(
    A_x, A_mem0, A_Wq, A_Wk, A_Wv, A_Wo, A_seg_len, B_x, B_w_in, B_w_sp, B_b_sp, B_w_out,
):
    assert A_x.shape == (1, S, D) and A_Wq.shape == (D, H, E) and B_w_in.shape == (D, 2 * FH)
    if isinstance(A_seg_len, int):
        assert A_seg_len == SEG
    hbm = pl.BlockSpec(memory_space=pl.ANY)
    out = pl.pallas_call(
        _kernel,
        out_shape=jax.ShapeDtypeStruct((S, D), BF16),
        in_specs=[hbm] * 10,
        out_specs=hbm,
        scratch_shapes=[
            pltpu.VMEM((S, D), BF16),
            pltpu.VMEM((S, D), F32),
            pltpu.VMEM((3, D * H, E), BF16),
            pltpu.VMEM((W_ROWS, E), U32),
            pltpu.VMEM((H * E, D), BF16),
            pltpu.VMEM((2 * FH, D), BF16),
            pltpu.VMEM((S, S), BF16),
            pltpu.VMEM((NT, FH, 128), F32),
            pltpu.VMEM((TPB, FH, 128), F32),
            pltpu.VMEM((NT, FH + 32, 128), BF16),
            pltpu.VMEM((128, FH), F32),
            pltpu.VMEM((S, D), BF16),
            pltpu.VMEM((2, len(MCH), 8, RB), F32),
            pltpu.VMEM((KVN, 2, M + 8, E), F32),
            pltpu.VMEM((FH, D), BF16),
            pltpu.VMEM((NT, 128), F32),
            pltpu.VMEM((M, D), BF16),
            pltpu.VMEM((NT, 128), BF16),
            pltpu.SemaphoreType.DMA((NSEM,)),
        ],
        compiler_params=pltpu.CompilerParams(vmem_limit_bytes=120 * 1024 * 1024),
    )(A_x.reshape(S, D), A_mem0.reshape(M, D), A_Wq.reshape(D * H, E), A_Wk.reshape(D * H, E),
      A_Wv.reshape(D * H, E), A_Wo.reshape(H * E, D), B_w_in.T, B_w_sp, B_b_sp.reshape(NT, 128), B_w_out)
    return out.reshape(1, S, D)
```
